```python
import jax
import jax.numpy as jnp

def _softmax(x, axis=-1):
    return jax.nn.softmax(x, axis=axis)
def _gelu(x):
    return jax.nn.gelu(x, approximate=True)
def _silu(x):
    return jax.nn.silu(x)
def _sigmoid(x):
    return jax.nn.sigmoid(x)
def _layernorm(x, axis=-1, eps=1e-5):
    m = jnp.mean(x, axis=axis, keepdims=True)
    v = jnp.var(x, axis=axis, keepdims=True)
    return (x - m) / jnp.sqrt(v + eps)
def _scatter_add(tgt, idx, src, axis=0):
    return tgt.at[idx].add(src)
def _segment_sum(src, seg, n):
    return jax.ops.segment_sum(src, seg, n)
class _Rng:
    def __init__(self, key):
        self._k = key
    def _next(self):
        self._k, sub = jax.random.split(self._k)
        return sub
    def normal(self, shape):
        return jax.random.normal(self._next(), shape, dtype=jnp.bfloat16)
    def randint(self, lo, hi, shape):
        return jax.random.randint(self._next(), shape, lo, hi, dtype=jnp.int32)
    def uniform(self, shape, lo=0.0, hi=1.0):
        return jax.random.uniform(self._next(), shape, jnp.bfloat16, lo, hi)
    def permutation(self, n):
        return jax.random.permutation(self._next(), n)


kernel_name = 'sequential_preLN__sliding_local_dilated__moe_arch_mod__prompt'

def setup_inputs():
    _rng = _Rng(jax.random.key(int.from_bytes(__import__("os").urandom(4), "little")))
    _w = (lambda a: (lambda t: t.astype(jnp.bfloat16) if jnp.issubdtype(t.dtype, jnp.floating) else t)(jnp.asarray(a)))
    def _A_setup():
        B, S, D = 1, 2048, 640
        return {
            "x": _w((lambda *s: _rng.normal(s) * 0.05)(B, S, D)),
            "wqkv": _w((lambda *s: _rng.normal(s) * 0.05)(D, 3 * D)),
            "wo": _w((lambda *s: _rng.normal(s) * 0.05)(D, D)),
        }
    _A_in = _A_setup()

    def _B_setup():
        B, S, D, F, C = 1, 2048, 640, 1536, 1
        return {
            "x": _w((lambda *s: _rng.normal(s) * 0.05)(B, S, D)),
            "w_r": _w((lambda *s: _rng.normal(s) * 0.05)(D)),
            "w_gate": _w((lambda *s: _rng.normal(s) * 0.05)(D, F)),
            "w_up": _w((lambda *s: _rng.normal(s) * 0.05)(D, F)),
            "w_down": _w((lambda *s: _rng.normal(s) * 0.05)(F, D)),
        }
    _B_in = _B_setup()

    return {
        "A_x": _A_in["x"],
        "A_wqkv": _A_in["wqkv"],
        "A_wo": _A_in["wo"],
        "B_x": _B_in["x"],
        "B_w_r": _B_in["w_r"],
        "B_w_gate": _B_in["w_gate"],
        "B_w_up": _B_in["w_up"],
        "B_w_down": _B_in["w_down"],
    }

def reference(A_x, A_wqkv, A_wo, B_x, B_w_r, B_w_gate, B_w_up, B_w_down):
    def _A_ref(x, wqkv, wo):
        B, S, D = x.shape
        H = 32; Dh = D // H
        W, dil = 8, 2
        qkv = (lambda x, *d: x.transpose(*d))((x @ wqkv).reshape(B, S, 3, H, Dh), 2, 0, 3, 1, 4)
        q, k, v = qkv[0], qkv[1], qkv[2]
        scale = Dh ** -0.5
        pos = jnp.arange(S)
        off = jnp.arange(W) * dil
        idx = pos[:, None] - off[None, :]
        mask = idx >= 0
        idx_c = jnp.where(mask, idx, 0).reshape(-1)
        kg = k[:, :, idx_c, :].reshape(B, H, S, W, Dh)
        vg = v[:, :, idx_c, :].reshape(B, H, S, W, Dh)
        logits = jnp.einsum("bhsd,bhswd->bhsw", q, kg) * scale
        logits = jnp.where(mask[None, None, :, :], logits, -1e9)
        attn = _softmax(logits, axis=-1)
        o = jnp.einsum("bhsw,bhswd->bhsd", attn, vg)
        return (lambda x, *d: x.transpose(*d))(o, 0, 2, 1, 3).reshape(B, S, D) @ wo

    def _B_ref(x, w_r, w_gate, w_up, w_down):
        B, S, D = x.shape
        C = 1
        r = x @ w_r
        idx = jnp.argsort(-r, axis=-1)[:, :C]
        idx_e = jnp.repeat(idx.reshape(B, C, 1), D, axis=2)
        x_sel = jnp.take_along_axis(x, idx_e, axis=1)
        g = _silu(x_sel @ w_gate)
        u = x_sel @ w_up
        y = (g * u) @ w_down
        r_sel = _sigmoid(jnp.take_along_axis(r, idx, axis=1))
        y = y * r_sel.reshape(B, C, 1)
        b_off = (jnp.arange(B) * S).reshape(B, 1)
        flat_idx = (idx + b_off).reshape(B * C)
        zero = (x * 0.0).reshape(B * S, D)
        upd = _scatter_add(zero, flat_idx, y.reshape(B * C, D), axis=0)
        return x + upd.reshape(B, S, D)

    x = A_x
    h = x + _A_ref(_layernorm(x, axis=-1), A_wqkv, A_wo)
    h2 = h + _B_ref(_layernorm(h, axis=-1), B_w_r, B_w_gate, B_w_up, B_w_down)
    return h2
```

```python
import functools
import jax
import jax.numpy as jnp
import numpy as np
import jax.experimental.pallas as pl
import jax.experimental.pallas.tpu as pltpu

S, D, H, DH, F = 2048, 640, 32, 20, 1536
NT = D // 128
WIN, DIL = 8, 2
HALO = 16
T = int(256)
NB = S // T
RA = int(32)
RL = int(32)
EPS = 1e-5
QSCALE = float(DH ** -0.5 * np.log2(np.e))


def _ln(x):
    m = jnp.sum(x, axis=-1, keepdims=True) * (1.0 / D)
    xc = x - m
    v = jnp.sum(xc * xc, axis=-1, keepdims=True) * (1.0 / D)
    return xc * jax.lax.rsqrt(v + EPS)


def _perm_rows(src_ref, kt, base, dst_store):
    for dp in range(DH // 2):
        a = src_ref[kt, pl.ds(base + dp, 16, stride=DH), :]
        b = src_ref[kt, pl.ds(base + dp + DH // 2, 16, stride=DH), :]
        dst_store(32 * dp, (a & jnp.uint32(0xFFFF)) | (b << 16))
        dst_store(32 * dp + 16, (a >> 16) | (b & jnp.uint32(0xFFFF0000)))


def _kernel(x_hbm, w_hbm, wo_hbm, wr_ref, wg_hbm, wu_hbm, wd_hbm, out_hbm,
            x_v, w_st, wt_tmp, wt_p, wo_st, wo_tmp, wo_p, ln_s, q_s, k_s, v_s, o_s, a_s, h_s, out_v,
            wg_v, wu_v, wd_v, xsem, wsem, fsem, osem):
    x_cp = [pltpu.make_async_copy(x_hbm.at[pl.ds(i * T, T), :], x_v.at[pl.ds(i * T, T), :], xsem.at[i])
            for i in range(NB)]
    w_cp = [pltpu.make_async_copy(w_hbm.at[pl.ds(kt * 128, 128), :], w_st.at[pl.ds(kt * 128, 128), :], wsem.at[kt])
            for kt in range(NT)]
    wo_cp = pltpu.make_async_copy(wo_hbm, wo_st, fsem.at[0])
    wg_cp = pltpu.make_async_copy(wg_hbm, wg_v, fsem.at[1])
    wu_cp = pltpu.make_async_copy(wu_hbm, wu_v, fsem.at[2])
    wd_cp = pltpu.make_async_copy(wd_hbm, wd_v, fsem.at[3])
    o_cp = [pltpu.make_async_copy(out_v.at[pl.ds(i * T, T), :], out_hbm.at[pl.ds(i * T, T), :], osem.at[i])
            for i in range(NB)]
    x_cp[0].start()
    for c in w_cp:
        c.start()
    x_cp[1].start()

    for a in range(NT):
        k_s[a, pl.ds(0, HALO), :] = jnp.zeros((HALO, 128), jnp.float32)
        v_s[a, pl.ds(0, HALO), :] = jnp.zeros((HALO, 128), jnp.float32)
    wr = wr_ref[...].reshape(1, D).astype(jnp.float32)

    zero_i = jax.lax.broadcasted_iota(jnp.int32, (8, 128), 1) >> 10
    chain = {'A': None, 'B': None}
    SC = int(1)
    XL = {'A': int(0), 'B': int(0)}

    def settok(v, ch='B'):
        t = pltpu.bitcast(jnp.broadcast_to(v[0:8, 0:128], (8, 128)), jnp.int32) & zero_i
        for _ in range(XL[ch]):
            t = pltpu.roll(t, 1, 1)
        chain['A' if SC else ch] = t

    def dep(x, ch='B'):
        tok = chain['A' if SC else ch]
        if tok is None:
            return x
        head = pltpu.bitcast(pltpu.bitcast(x[0:8], jnp.int32) | tok, jnp.float32)
        return jnp.concatenate([head, x[8:]], axis=0) if x.shape[0] > 8 else head

    def lsum(xs):
        return jnp.sum(functools.reduce(jnp.add, xs), axis=-1, keepdims=True)

    def stats(xs):
        s1 = lsum(xs)
        s2 = lsum([x * x for x in xs])
        m = s1 * (1.0 / D)
        var = jnp.maximum(s2 * (1.0 / D) - m * m, 0.0)
        return m, jax.lax.rsqrt(var + EPS)

    def ln1c(i, c):
        r = i * T + c * RL
        xs = [x_v[pl.ds(r, RL), pl.ds(a * 128, 128)].astype(jnp.float32) for a in range(NT)]
        xs[0] = dep(xs[0])
        m, rs = stats(xs)
        settok(rs if TP == 0 else m)
        for a in range(NT):
            ln_s[pl.ds(r, RL), pl.ds(a * 128, 128)] = ((xs[a] - m) * rs).astype(jnp.bfloat16)
    TP = int(1)

    def prep_w():
        for kt in range(NT):
            w_cp[kt].wait()
            wt = w_st[pl.ds(kt * 128, 128), :].T
            wt_tmp[kt] = pltpu.bitcast(wt, jnp.uint32)
            for part in range(3):
                def st(r, val, kt=kt, part=part):
                    wt_p[pl.ds(part * 320 + r, 16), pl.ds(kt * 128, 128)] = val
                _perm_rows(wt_tmp, kt, part * 320, st)

    def prep_wo():
        wo_cp.wait()
        for nt in range(NT):
            wo_tmp[nt] = pltpu.bitcast(wo_st[:, pl.ds(nt * 128, 128)], jnp.uint32)
        for nt in range(NT):
            def st(r, val, nt=nt):
                wo_p[pl.ds(r, 16), pl.ds(nt * 128, 128)] = val
            _perm_rows(wo_tmp, nt, 0, st)

    def qkv(i):
        lhs = ln_s[pl.ds(i * T, T), :]
        for part, dst in ((1, k_s), (0, q_s), (2, v_s)):
            wt = pltpu.bitcast(wt_p[pl.ds(part * 320, 320), :], jnp.bfloat16)
            y = jax.lax.dot_general(lhs, wt, (((1,), (1,)), ((), ())), preferred_element_type=jnp.float32)
            for a in range(NT):
                ya = y[:, a * 128:(a + 1) * 128]
                if part == 0:
                    q_s[i % 2, a] = ya
                else:
                    dst[a, pl.ds(HALO + i * T, T), :] = ya

    CH = int(2)

    def attc(i, c):
            r = i * T + c * RA
            q = [q_s[i % 2, a, pl.ds(c * RA, RA), :] * QSCALE for a in range(NT)]
            q[0] = dep(q[0], 'A')
            ps = []
            for w in range(WIN):
                p = None
                for a in range(NT):
                    t = q[a] * k_s[a, pl.ds(HALO + r - DIL * w, RA), :]
                    p = t if p is None else p + t
                ps.append(p)
            ts = [pltpu.roll(p, 64, 1) for p in ps]
            if CH == 3:
                settok(ps[-1], 'A')
            ps = [p + t for p, t in zip(ps, ts)]
            ts = [pltpu.roll(p, 32, 1) for p in ps]
            if CH == 5:
                settok(ps[-1], 'A')
            ls = []
            for w, (p, t) in enumerate(zip(ps, ts)):
                p = p + t
                if r < DIL * w:
                    row = r + jax.lax.broadcasted_iota(jnp.int32, (RA, 128), 0)
                    p = jnp.where(row >= DIL * w, p, -1e30)
                ls.append(p)
            m = functools.reduce(jnp.maximum, ls)
            if CH == 4:
                settok(m, 'A')
            es = [jnp.exp2(l - m) for l in ls]
            inv = pl.reciprocal(functools.reduce(jnp.add, es))
            if CH == 2:
                settok(inv, 'A')
            for a in range(NT):
                o = None
                for w in range(WIN):
                    t = es[w] * v_s[a, pl.ds(HALO + r - DIL * w, RA), :]
                    o = t if o is None else o + t
                o_s[i % 2, pl.ds(c * RA, RA), a * 128:(a + 1) * 128] = (o * inv).astype(jnp.bfloat16)
            if CH == 1:
                settok(o, 'A')

    def wo_mm(i):
        wo = pltpu.bitcast(wo_p[...], jnp.bfloat16)
        a_s[i % 2] = jnp.dot(o_s[i % 2], wo, preferred_element_type=jnp.float32)

    st = {'best': jnp.full((RL, 1), -jnp.inf, jnp.float32), 'besti': jnp.zeros((RL, 1), jnp.int32)}

    wrs = [jnp.broadcast_to(wr[:, a * 128:(a + 1) * 128], (RL, 128)) for a in range(NT)]
    wsum = jnp.sum(wr, axis=-1, keepdims=True)

    def postc(i, c):
            r = i * T + c * RL
            xs = [x_v[pl.ds(r, RL), pl.ds(a * 128, 128)].astype(jnp.float32) for a in range(NT)]
            xs[0] = dep(xs[0])
            hs = [xs[a] + a_s[i % 2, pl.ds(c * RL, RL), pl.ds(a * 128, 128)] for a in range(NT)]
            for a in range(NT):
                h_s[a, pl.ds(r, RL), :] = hs[a]
            s3 = lsum([h * w for h, w in zip(hs, wrs)])
            m, rs = stats(hs)
            settok(rs if TP == 0 else m)
            rr = rs * (s3 - m * wsum)
            rowi = r + jax.lax.broadcasted_iota(jnp.int32, (RL, 1), 0)
            upd = rr > st['best']
            st['best'] = jnp.where(upd, rr, st['best'])
            st['besti'] = jnp.where(upd, rowi, st['besti'])
            for a in range(NT):
                out_v[pl.ds(r, RL), pl.ds(a * 128, 128)] = (hs[a] + (hs[a] - m) * rs).astype(jnp.bfloat16)

    x_cp[0].wait()
    for c in range(T // RL):
        ln1c(0, c)
    prep_w()
    wo_cp.start()
    NC = T // RA
    for i in range(NB + 3):
        if i + 2 < NB:
            x_cp[i + 2].start()
        if i + 1 < NB:
            x_cp[i + 1].wait()
        if 4 <= i:
            o_cp[i - 4].start()
        if i == 2:
            wg_cp.start()
            wu_cp.start()
            wd_cp.start()
        if i == 1:
            prep_wo()
        if 2 <= i < NB + 2:
            wo_mm(i - 2)
        if i < NB:
            qkv(i)
        for c in range(NC):
            if 1 <= i <= NB:
                attc(i - 1, c)
            if (c + 1) * RA % RL == 0:
                c2 = (c + 1) * RA // RL - 1
                if 3 <= i:
                    postc(i - 3, c2)
                if i + 1 < NB:
                    ln1c(i + 1, c2)
    o_cp[NB - 1].start()
    best, besti = st['best'], st['besti']

    rmax = jnp.max(best)
    idx = jnp.min(jnp.where(best == rmax, besti, S))
    idx = jnp.clip(idx, 0, S - 1)
    hrow = jnp.concatenate([h_s[a, pl.ds(idx, 1), :] for a in range(NT)], axis=1)
    ln2row = _ln(hrow)
    xs = jnp.broadcast_to(ln2row, (16, D)).astype(jnp.bfloat16)
    wg_cp.wait()
    wu_cp.wait()
    wd_cp.wait()
    g = jnp.dot(xs, wg_v[...], preferred_element_type=jnp.float32)
    u = jnp.dot(xs, wu_v[...], preferred_element_type=jnp.float32)
    act = (g * jax.nn.sigmoid(g) * u).astype(jnp.bfloat16)
    y = jnp.dot(act, wd_v[...], preferred_element_type=jnp.float32)
    y = y * jax.nn.sigmoid(jnp.full((16, D), rmax, jnp.float32))
    newrow = hrow + ln2row + y[0:1]
    for i in range(NB):
        o_cp[i].wait()
    base = pl.multiple_of((idx // 16) * 16, 16)
    tile = out_v[pl.ds(base, 16), :].astype(jnp.float32)
    rr = base + jax.lax.broadcasted_iota(jnp.int32, (16, D), 0)
    tile = jnp.where(rr == idx, jnp.broadcast_to(newrow, (16, D)), tile)
    out_v[pl.ds(base, 16), :] = tile.astype(jnp.bfloat16)
    cp = pltpu.make_async_copy(out_v.at[pl.ds(base, 16), :], out_hbm.at[pl.ds(base, 16), :], osem.at[0])
    cp.start()
    cp.wait()


@jax.jit
def pallas_sequential_preLN__sliding_local_dilated__moe_arch_mod__prompt_kernel(
    A_x, A_wqkv, A_wo, B_x, B_w_r, B_w_gate, B_w_up, B_w_down,
):
    del B_x
    any_spec = pl.BlockSpec(memory_space=pl.ANY)
    out = pl.pallas_call(
        _kernel,
        out_shape=jax.ShapeDtypeStruct((S, D), jnp.bfloat16),
        in_specs=[any_spec, any_spec, any_spec, pl.BlockSpec(memory_space=pltpu.VMEM),
                  any_spec, any_spec, any_spec],
        out_specs=any_spec,
        scratch_shapes=[
            pltpu.VMEM((S, D), jnp.bfloat16),
            pltpu.VMEM((D, 3 * D), jnp.bfloat16),
            pltpu.VMEM((NT, 960, 128), jnp.uint32),
            pltpu.VMEM((960, D), jnp.uint32),
            pltpu.VMEM((D, D), jnp.bfloat16),
            pltpu.VMEM((NT, 320, 128), jnp.uint32),
            pltpu.VMEM((320, D), jnp.uint32),
            pltpu.VMEM((S, D), jnp.bfloat16),
            pltpu.VMEM((2, NT, T, 128), jnp.float32),
            pltpu.VMEM((NT, HALO + S, 128), jnp.float32),
            pltpu.VMEM((NT, HALO + S, 128), jnp.float32),
            pltpu.VMEM((2, T, D), jnp.bfloat16),
            pltpu.VMEM((2, T, D), jnp.float32),
            pltpu.VMEM((NT, S, 128), jnp.float32),
            pltpu.VMEM((S, D), jnp.bfloat16),
            pltpu.VMEM((D, F), jnp.bfloat16),
            pltpu.VMEM((D, F), jnp.bfloat16),
            pltpu.VMEM((F, D), jnp.bfloat16),
            pltpu.SemaphoreType.DMA((NB,)),
            pltpu.SemaphoreType.DMA((NT,)),
            pltpu.SemaphoreType.DMA((4,)),
            pltpu.SemaphoreType.DMA((NB,)),
        ],
        compiler_params=pltpu.CompilerParams(vmem_limit_bytes=100 * 1024 * 1024),
    )(A_x.reshape(S, D), A_wqkv, A_wo, B_w_r, B_w_gate, B_w_up, B_w_down)
    return out.reshape(1, S, D)
```

```python
import functools
import jax
import jax.numpy as jnp
import numpy as np
import jax.experimental.pallas as pl
import jax.experimental.pallas.tpu as pltpu

S, D, H, DH, F = 2048, 640, 32, 20, 1536
NT = D // 128
WIN, DIL = 8, 2
HALO = 16
RA = int(32)
NCK = S // RA
EPS = 1e-5
QSCALE = float(DH ** -0.5 * np.log2(np.e))
BLOCKS = [int(v) for v in '256,128,128,128,128,128,128,128,128,128,128,128,128,64,64,64,64'.split(',')]
assert sum(BLOCKS) == S
STARTS = [sum(BLOCKS[:i]) for i in range(len(BLOCKS))]
NBK = len(BLOCKS)
XB = 256
NX = S // XB
CH = int(2)
TP = int(1)
WF = int(1)
LA = int(8)
LP = int(2)
BND = [int(v) for v in '2,5,8,13'.split(',')]


def _perm_rows(src_ref, kt, base, dst_store):
    for dp in range(DH // 2):
        a = src_ref[kt, pl.ds(base + dp, 16, stride=DH), :]
        b = src_ref[kt, pl.ds(base + dp + DH // 2, 16, stride=DH), :]
        dst_store(32 * dp, (a & jnp.uint32(0xFFFF)) | (b << 16))
        dst_store(32 * dp + 16, (a >> 16) | (b & jnp.uint32(0xFFFF0000)))


def _kernel(x_hbm, w_hbm, wo_hbm, wr_ref, wg_hbm, wu_hbm, wd_hbm, out_hbm,
            x_v, w_st, wt_tmp, wt_p, wo_st, wo_tmp, wo_p, ln_s, q_s, k_s, v_s, o_s, h_s, out_v,
            wg_v, wu_v, wd_v, xsem, wsem, fsem, osem):
    x_cp = [pltpu.make_async_copy(x_hbm.at[pl.ds(i * XB, XB), :], x_v.at[pl.ds(i * XB, XB), :], xsem.at[i])
            for i in range(NX)]
    w_cp = [pltpu.make_async_copy(w_hbm.at[pl.ds(kt * 128, 128), :], w_st.at[pl.ds(kt * 128, 128), :], wsem.at[kt])
            for kt in range(NT)]
    wo_cp = pltpu.make_async_copy(wo_hbm, wo_st, fsem.at[0])
    wg_cp = pltpu.make_async_copy(wg_hbm, wg_v, fsem.at[1])
    wu_cp = pltpu.make_async_copy(wu_hbm, wu_v, fsem.at[2])
    wd_cp = pltpu.make_async_copy(wd_hbm, wd_v, fsem.at[3])
    o_cp = [pltpu.make_async_copy(out_v.at[pl.ds(i * XB, XB), :], out_hbm.at[pl.ds(i * XB, XB), :], osem.at[i])
            for i in range(NX)]
    x_cp[0].start()
    for c in w_cp:
        c.start()
    x_cp[1].start()

    for a in range(NT):
        k_s[a, pl.ds(0, HALO), :] = jnp.zeros((HALO, 128), jnp.float32)
        v_s[a, pl.ds(0, HALO), :] = jnp.zeros((HALO, 128), jnp.float32)
    wr = wr_ref[...].reshape(1, D).astype(jnp.float32)
    wrs = [jnp.broadcast_to(wr[:, a * 128:(a + 1) * 128], (RA, 128)) for a in range(NT)]
    wsum = jnp.sum(wr, axis=-1, keepdims=True)

    zero_i = jax.lax.broadcasted_iota(jnp.int32, (8, 128), 1) >> 10
    chain = {'t': None}

    def settok(v):
        chain['t'] = pltpu.bitcast(jnp.broadcast_to(v[0:8, 0:128], (8, 128)), jnp.int32) & zero_i

    def dep(x):
        tok = chain['t']
        if tok is None:
            return x
        head = pltpu.bitcast(pltpu.bitcast(x[0:8], jnp.int32) | tok, jnp.float32)
        return jnp.concatenate([head, x[8:]], axis=0)

    LQ = int(0)
    LV = int(0)

    def link(x, prev):
        t = zero_i
        for g in range(prev.shape[0] // 8):
            t = t & pltpu.bitcast(prev[g * 8:(g + 1) * 8], jnp.int32)
        head = pltpu.bitcast(pltpu.bitcast(x[0:8], jnp.int32) | t, jnp.float32)
        return jnp.concatenate([head, x[8:]], axis=0)

    def lsum(xs):
        return jnp.sum(functools.reduce(jnp.add, xs), axis=-1, keepdims=True)

    def rsq(x):
        return jnp.exp2(jnp.log2(x) * -0.5)

    def stats(xs):
        s1 = lsum(xs)
        s2 = lsum([x * x for x in xs])
        m = s1 * (1.0 / D)
        var = jnp.maximum(s2 * (1.0 / D) - m * m, 0.0)
        return m, rsq(var + EPS)

    def xtiles(r):
        return [x_v[pl.ds(r, RA), pl.ds(a * 128, 128)].astype(jnp.float32) for a in range(NT)]

    def ln1c(j):
        r = j * RA
        xs = xtiles(r)
        xs[0] = dep(xs[0])
        m, rs = stats(xs)
        settok(rs if TP == 0 else m)
        for a in range(NT):
            ln_s[pl.ds(r // 2, RA // 2), pl.ds(a * 128, 128)] = pltpu.bitcast(
                ((xs[a] - m) * rs).astype(jnp.bfloat16), jnp.uint32)

    def prep_w(kt):
        wt = w_st[pl.ds(kt * 128, 128), :].T
        wt_tmp[kt] = pltpu.bitcast(wt, jnp.uint32)
        for part in range(3):
            def st(r, val, part=part):
                wt_p[pl.ds(part * 320 + r, 16), pl.ds(kt * 128, 128)] = val
            _perm_rows(wt_tmp, kt, part * 320, st)

    def qkv0_part(kt):
        n = BLOCKS[0]
        lhs = pltpu.bitcast(ln_s[pl.ds(0, n // 2), pl.ds(kt * 128, 128)], jnp.bfloat16)
        for part, dst, off in ((1, k_s, HALO), (0, q_s, 0), (2, v_s, HALO)):
            wt = pltpu.bitcast(wt_p[pl.ds(part * 320, 320), pl.ds(kt * 128, 128)], jnp.bfloat16)
            y = jax.lax.dot_general(lhs, wt, (((1,), (1,)), ((), ())), preferred_element_type=jnp.float32)
            for a in range(NT):
                if kt == 0:
                    dst[a, pl.ds(off, n), :] = y[:, a * 128:(a + 1) * 128]
                else:
                    dst[a, pl.ds(off, n), :] += y[:, a * 128:(a + 1) * 128]

    def prep_wo():
        for nt in range(NT):
            wo_tmp[nt] = pltpu.bitcast(wo_st[:, pl.ds(nt * 128, 128)], jnp.uint32)
        for nt in range(NT):
            def st(r, val, nt=nt):
                wo_p[pl.ds(r, 16), pl.ds(nt * 128, 128)] = val
            _perm_rows(wo_tmp, nt, 0, st)

    def qkv(b):
        s0, n = STARTS[b], BLOCKS[b]
        lhs = pltpu.bitcast(ln_s[pl.ds(s0 // 2, n // 2), :], jnp.bfloat16)
        for part, dst, off in ((1, k_s, HALO), (0, q_s, 0), (2, v_s, HALO)):
            wt = pltpu.bitcast(wt_p[pl.ds(part * 320, 320), :], jnp.bfloat16)
            y = jax.lax.dot_general(lhs, wt, (((1,), (1,)), ((), ())), preferred_element_type=jnp.float32)
            for a in range(NT):
                dst[a, pl.ds(off + s0, n), :] = y[:, a * 128:(a + 1) * 128]

    def attc(j):
        r = j * RA
        q = [q_s[a, pl.ds(r, RA), :] * QSCALE for a in range(NT)]
        q[0] = dep(q[0])
        ps = []
        for w in range(WIN):
            p = None
            for a in range(NT):
                kk = k_s[a, pl.ds(HALO + r - DIL * w, RA), :]
                if a == 0 and LQ and w % LQ == 0 and w > 0:
                    kk = link(kk, ps[-1])
                t = q[a] * kk
                p = t if p is None else p + t
            ps.append(p)
        ts = [pltpu.roll(p, 64, 1) for p in ps]
        ps = [p + t for p, t in zip(ps, ts)]
        ts = [pltpu.roll(p, 32, 1) for p in ps]
        ls = []
        for w, (p, t) in enumerate(zip(ps, ts)):
            p = p + t
            if r < DIL * w:
                row = r + jax.lax.broadcasted_iota(jnp.int32, (RA, 128), 0)
                p = jnp.where(row >= DIL * w, p, -1e30)
            ls.append(p)
        m = functools.reduce(jnp.maximum, ls)
        if CH == 4:
            settok(m)
        es = [jnp.exp2(l - m) for l in ls]
        inv = pl.reciprocal(functools.reduce(jnp.add, es), approx=True)
        if CH == 2:
            settok(inv)
        oprev = None
        for a in range(NT):
            o = None
            for w in range(WIN):
                vv = v_s[a, pl.ds(HALO + r - DIL * w, RA), :]
                if w == 0 and LV and oprev is not None:
                    vv = link(vv, oprev)
                t = es[w] * vv
                o = t if o is None else o + t
            oprev = o
            o_s[pl.ds(r // 2, RA // 2), pl.ds(a * 128, 128)] = pltpu.bitcast(
                (o * inv).astype(jnp.bfloat16), jnp.uint32)
        if CH == 1:
            settok(o)

    def wo_mm(b):
        s0, n = STARTS[b], BLOCKS[b]
        wo = pltpu.bitcast(wo_p[...], jnp.bfloat16)
        lhs = pltpu.bitcast(o_s[pl.ds(s0 // 2, n // 2), :], jnp.bfloat16)
        y = jnp.dot(lhs, wo, preferred_element_type=jnp.float32)
        for a in range(NT):
            h_s[a, pl.ds(s0, n), :] = y[:, a * 128:(a + 1) * 128]

    st = {'best': jnp.full((RA, 1), -jnp.inf, jnp.float32), 'besti': jnp.zeros((RA, 1), jnp.int32)}

    def postc(j):
        r = j * RA
        xs = xtiles(r)
        xs[0] = dep(xs[0])
        hs = [xs[a] + h_s[a, pl.ds(r, RA), :] for a in range(NT)]
        for a in range(NT):
            h_s[a, pl.ds(r, RA), :] = hs[a]
        s3 = lsum([h * w for h, w in zip(hs, wrs)])
        m, rs = stats(hs)
        settok(rs if TP == 0 else m)
        rr = rs * (s3 - m * wsum)
        rowi = r + jax.lax.broadcasted_iota(jnp.int32, (RA, 1), 0)
        upd = rr > st['best']
        st['best'] = jnp.where(upd, rr, st['best'])
        st['besti'] = jnp.where(upd, rowi, st['besti'])
        for a in range(NT):
            out_v[pl.ds(r, RA), pl.ds(a * 128, 128)] = (hs[a] + (hs[a] - m) * rs).astype(jnp.bfloat16)

    def blk(j):
        r = j * RA
        return max(b for b in range(NBK) if STARTS[b] <= r)

    x_cp[0].wait()
    nl = 0
    while nl * RA < BLOCKS[0]:
        ln1c(nl)
        chain['t'] = None
        nl += 1
    for kt in range(NT + 1):
        if kt < NT:
            w_cp[kt].wait()
        if kt == int(2):
            x_cp[2].start()
            wo_cp.start()
            x_cp[3].start()
        if kt == NT:
            for jx in range(4, NX):
                x_cp[jx].start()
        if kt == NT:
            x_cp[1].wait()
        if kt > 0:
            qkv0_part(kt - 1)
        if kt < NT:
            prep_w(kt)
    xw = 2
    npost = 0
    nout = 0
    waited_o = 0
    na = 0
    nbnd = 0
    for b in range(1, NBK + 1):
        if b in BND:
            while (nout + 1) * XB <= npost * RA:
                o_cp[nout].start()
                nout += 1
            if nbnd == 0:
                wo_cp.wait()
                while xw < 4:
                    x_cp[xw].wait()
                    xw += 1
                prep_wo()
            elif nbnd == 1:
                while xw < NX:
                    x_cp[xw].wait()
                    xw += 1
                wg_cp.start()
                wu_cp.start()
                wd_cp.start()
            else:
                assert waited_o < nout - 1
                o_cp[waited_o].wait()
                waited_o += 1
            nbnd += 1
        if b >= 2:
            assert nbnd >= 1
            wo_mm(b - 2)
        if b < NBK:
            while nl * RA < STARTS[b] + BLOCKS[b]:
                ln1c(nl)
                nl += 1
            qkv(b)
        nck = BLOCKS[b - 1] // RA
        for c in range(nck):
            attc(na)
            na += 1
            lim = max(0, na - BLOCKS[max(b - 2, 0)] // RA - LP) if b >= 2 else 0
            lim = min(lim, STARTS[b - 1] // RA)
            want_ln = min(xw * XB // RA, na + LA)
            k = 0
            if npost < lim:
                postc(npost)
                npost += 1
                k += 1
            if nl < want_ln:
                ln1c(nl)
                nl += 1
                k += 1
            if k < 2 and npost < lim:
                postc(npost)
                npost += 1
        assert nl * RA <= xw * XB
    wo_mm(NBK - 1)
    while npost < NCK:
        postc(npost)
        npost += 1
    while nout < NX:
        o_cp[nout].start()
        nout += 1
    best, besti = st['best'], st['besti']

    rmax = jnp.max(best)
    idx = jnp.min(jnp.where(best == rmax, besti, S))
    idx = jnp.clip(idx, 0, S - 1)
    hrow = [h_s[a, pl.ds(idx, 1), :] for a in range(NT)]
    m, rs = stats(hrow)
    hrow = jnp.concatenate(hrow, axis=1)
    ln2row = (hrow - m) * rs
    xs = jnp.broadcast_to(ln2row, (16, D)).astype(jnp.bfloat16)
    wg_cp.wait()
    wu_cp.wait()
    wd_cp.wait()
    g = jnp.dot(xs, wg_v[...], preferred_element_type=jnp.float32)
    u = jnp.dot(xs, wu_v[...], preferred_element_type=jnp.float32)
    act = (g * jax.nn.sigmoid(g) * u).astype(jnp.bfloat16)
    y = jnp.dot(act, wd_v[...], preferred_element_type=jnp.float32)
    y = y * jax.nn.sigmoid(jnp.full((16, D), rmax, jnp.float32))
    newrow = hrow + ln2row + y[0:1]
    for i in range(waited_o, NX):
        o_cp[i].wait()
    base = pl.multiple_of((idx // 16) * 16, 16)
    tile = out_v[pl.ds(base, 16), :].astype(jnp.float32)
    rr = base + jax.lax.broadcasted_iota(jnp.int32, (16, D), 0)
    tile = jnp.where(rr == idx, jnp.broadcast_to(newrow, (16, D)), tile)
    out_v[pl.ds(base, 16), :] = tile.astype(jnp.bfloat16)
    cp = pltpu.make_async_copy(out_v.at[pl.ds(base, 16), :], out_hbm.at[pl.ds(base, 16), :], osem.at[0])
    cp.start()
    cp.wait()


@jax.jit
def pallas_sequential_preLN__sliding_local_dilated__moe_arch_mod__prompt_kernel(
    A_x, A_wqkv, A_wo, B_x, B_w_r, B_w_gate, B_w_up, B_w_down,
):
    del B_x
    any_spec = pl.BlockSpec(memory_space=pl.ANY)
    out = pl.pallas_call(
        _kernel,
        out_shape=jax.ShapeDtypeStruct((S, D), jnp.bfloat16),
        in_specs=[any_spec, any_spec, any_spec, pl.BlockSpec(memory_space=pltpu.VMEM),
                  any_spec, any_spec, any_spec],
        out_specs=any_spec,
        scratch_shapes=[
            pltpu.VMEM((S, D), jnp.bfloat16),
            pltpu.VMEM((D, 3 * D), jnp.bfloat16),
            pltpu.VMEM((NT, 960, 128), jnp.uint32),
            pltpu.VMEM((960, D), jnp.uint32),
            pltpu.VMEM((D, D), jnp.bfloat16),
            pltpu.VMEM((NT, 320, 128), jnp.uint32),
            pltpu.VMEM((320, D), jnp.uint32),
            pltpu.VMEM((S // 2, D), jnp.uint32),
            pltpu.VMEM((NT, S, 128), jnp.float32),
            pltpu.VMEM((NT, HALO + S, 128), jnp.float32),
            pltpu.VMEM((NT, HALO + S, 128), jnp.float32),
            pltpu.VMEM((S // 2, D), jnp.uint32),
            pltpu.VMEM((NT, S, 128), jnp.float32),
            pltpu.VMEM((S, D), jnp.bfloat16),
            pltpu.VMEM((D, F), jnp.bfloat16),
            pltpu.VMEM((D, F), jnp.bfloat16),
            pltpu.VMEM((F, D), jnp.bfloat16),
            pltpu.SemaphoreType.DMA((NX,)),
            pltpu.SemaphoreType.DMA((NT,)),
            pltpu.SemaphoreType.DMA((4,)),
            pltpu.SemaphoreType.DMA((NX,)),
        ],
        compiler_params=pltpu.CompilerParams(vmem_limit_bytes=100 * 1024 * 1024),
    )(A_x.reshape(S, D), A_wqkv, A_wo, B_w_r, B_w_gate, B_w_up, B_w_down)
    return out.reshape(1, S, D)
```

```python
import functools
import jax
import jax.numpy as jnp
import numpy as np
import jax.experimental.pallas as pl
import jax.experimental.pallas.tpu as pltpu

S, D, H, DH, F = 2048, 640, 32, 20, 1536
NT = D // 128
WIN, DIL = 8, 2
HALO = 16
RA = int(32)
NCK = S // RA
EPS = 1e-5
QSCALE = float(DH ** -0.5 * np.log2(np.e))
BLOCKS = [int(v) for v in '256,128,128,128,128,128,128,128,128,128,128,128,128,64,64,64,64'.split(',')]
assert sum(BLOCKS) == S
STARTS = [sum(BLOCKS[:i]) for i in range(len(BLOCKS))]
NBK = len(BLOCKS)
XB = 256
NX = S // XB
CH = int(2)
TP = int(1)
WF = int(1)
LA = int(10)
DT = int(1)
LC = int(9)
KM = int(2)
LP = int(2)
BND = [int(v) for v in '1,4,9,15'.split(',')]


def _perm_rows(src_ref, kt, base, dst_store):
    for dp in range(DH // 2):
        a = src_ref[kt, pl.ds(base + dp, 16, stride=DH), :]
        b = src_ref[kt, pl.ds(base + dp + DH // 2, 16, stride=DH), :]
        dst_store(32 * dp, (a & jnp.uint32(0xFFFF)) | (b << 16))
        dst_store(32 * dp + 16, (a >> 16) | (b & jnp.uint32(0xFFFF0000)))


def _kernel(x_hbm, w_hbm, wo_hbm, wr_ref, wg_hbm, wu_hbm, wd_hbm, out_hbm,
            x_v, w_st, wt_tmp, wt_p, wo_st, wo_tmp, wo_p, ln_s, q_s, k_s, v_s, o_s, h_s, out_v,
            wg_v, wu_v, wd_v, xsem, wsem, fsem, osem):
    x_cp = [pltpu.make_async_copy(x_hbm.at[pl.ds(i * XB, XB), :], x_v.at[pl.ds(i * XB, XB), :], xsem.at[i])
            for i in range(NX)]
    w_cp = [pltpu.make_async_copy(w_hbm.at[pl.ds(kt * 128, 128), :], w_st.at[pl.ds(kt * 128, 128), :], wsem.at[kt])
            for kt in range(NT)]
    wo_cp = pltpu.make_async_copy(wo_hbm, wo_st, fsem.at[0])
    wg_cp = pltpu.make_async_copy(wg_hbm, wg_v, fsem.at[1])
    wu_cp = pltpu.make_async_copy(wu_hbm, wu_v, fsem.at[2])
    wd_cp = pltpu.make_async_copy(wd_hbm, wd_v, fsem.at[3])
    o_cp = [pltpu.make_async_copy(out_v.at[pl.ds(i * XB, XB), :], out_hbm.at[pl.ds(i * XB, XB), :], osem.at[i])
            for i in range(NX)]
    x_cp[0].start()
    for c in w_cp:
        c.start()
    x_cp[1].start()

    for a in range(NT):
        k_s[a, pl.ds(0, HALO), :] = jnp.zeros((HALO, 128), jnp.float32)
        v_s[a, pl.ds(0, HALO), :] = jnp.zeros((HALO, 128), jnp.float32)
    wr = wr_ref[...].reshape(1, D).astype(jnp.float32)
    wrs = [jnp.broadcast_to(wr[:, a * 128:(a + 1) * 128], (RA, 128)) for a in range(NT)]
    wsum = jnp.sum(wr, axis=-1, keepdims=True)

    zero_i = jax.lax.broadcasted_iota(jnp.int32, (8, 128), 1) >> 10
    chain = {'t': None}

    def settok(v):
        chain['t'] = pltpu.bitcast(jnp.broadcast_to(v[0:8, 0:128], (8, 128)), jnp.int32) & zero_i

    def dep(x):
        tok = chain['t']
        if tok is None:
            return x
        head = pltpu.bitcast(pltpu.bitcast(x[0:8], jnp.int32) | tok, jnp.float32)
        return jnp.concatenate([head, x[8:]], axis=0)

    LQ = int(0)
    LV = int(0)

    def link(x, prev):
        t = zero_i
        for g in range(prev.shape[0] // 8):
            t = t & pltpu.bitcast(prev[g * 8:(g + 1) * 8], jnp.int32)
        head = pltpu.bitcast(pltpu.bitcast(x[0:8], jnp.int32) | t, jnp.float32)
        return jnp.concatenate([head, x[8:]], axis=0)

    def lsum(xs):
        return jnp.sum(functools.reduce(jnp.add, xs), axis=-1, keepdims=True)

    def rsq(x):
        return jnp.exp2(jnp.log2(x) * -0.5)

    def stats(xs):
        s1 = lsum(xs)
        s2 = lsum([x * x for x in xs])
        m = s1 * (1.0 / D)
        var = jnp.maximum(s2 * (1.0 / D) - m * m, 0.0)
        return m, rsq(var + EPS)

    def xtiles(r):
        return [x_v[pl.ds(r, RA), pl.ds(a * 128, 128)].astype(jnp.float32) for a in range(NT)]

    def ln1c(j):
        r = j * RA
        xs = xtiles(r)
        xs[0] = dep(xs[0])
        m, rs = stats(xs)
        settok(rs if TP == 0 else m)
        for a in range(NT):
            ln_s[pl.ds(r // 2, RA // 2), pl.ds(a * 128, 128)] = pltpu.bitcast(
                ((xs[a] - m) * rs).astype(jnp.bfloat16), jnp.uint32)

    def prep_w(kt):
        wt = w_st[pl.ds(kt * 128, 128), :].T
        wt_tmp[kt] = pltpu.bitcast(wt, jnp.uint32)
        for part in range(3):
            def st(r, val, part=part):
                wt_p[pl.ds(part * 320 + r, 16), pl.ds(kt * 128, 128)] = val
            _perm_rows(wt_tmp, kt, part * 320, st)

    def qkv0_part(kt):
        n = BLOCKS[0]
        lhs = pltpu.bitcast(ln_s[pl.ds(0, n // 2), pl.ds(kt * 128, 128)], jnp.bfloat16)
        for part, dst, off in ((1, k_s, HALO), (0, q_s, 0), (2, v_s, HALO)):
            wt = pltpu.bitcast(wt_p[pl.ds(part * 320, 320), pl.ds(kt * 128, 128)], jnp.bfloat16)
            y = jax.lax.dot_general(lhs, wt, (((1,), (1,)), ((), ())), preferred_element_type=jnp.float32)
            for a in range(NT):
                if kt == 0:
                    dst[a, pl.ds(off, n), :] = y[:, a * 128:(a + 1) * 128]
                else:
                    dst[a, pl.ds(off, n), :] += y[:, a * 128:(a + 1) * 128]

    def prep_wo():
        for nt in range(NT):
            wo_tmp[nt] = pltpu.bitcast(wo_st[:, pl.ds(nt * 128, 128)], jnp.uint32)
        for nt in range(NT):
            def st(r, val, nt=nt):
                wo_p[pl.ds(r, 16), pl.ds(nt * 128, 128)] = val
            _perm_rows(wo_tmp, nt, 0, st)

    def qkv(b):
        s0, n = STARTS[b], BLOCKS[b]
        lhs = pltpu.bitcast(ln_s[pl.ds(s0 // 2, n // 2), :], jnp.bfloat16)
        for part, dst, off in ((1, k_s, HALO), (0, q_s, 0), (2, v_s, HALO)):
            wt = pltpu.bitcast(wt_p[pl.ds(part * 320, 320), :], jnp.bfloat16)
            y = jax.lax.dot_general(lhs, wt, (((1,), (1,)), ((), ())), preferred_element_type=jnp.float32)
            for a in range(NT):
                dst[a, pl.ds(off + s0, n), :] = y[:, a * 128:(a + 1) * 128]

    def attc(j):
        r = j * RA
        q = [q_s[a, pl.ds(r, RA), :] * QSCALE for a in range(NT)]
        q[0] = dep(q[0])
        ps = []
        for w in range(WIN):
            p = None
            for a in range(NT):
                kk = k_s[a, pl.ds(HALO + r - DIL * w, RA), :]
                if a == 0 and LQ and w % LQ == 0 and w > 0:
                    kk = link(kk, ps[-1])
                t = q[a] * kk
                p = t if p is None else p + t
            ps.append(p)
        ts = [pltpu.roll(p, 64, 1) for p in ps]
        ps = [p + t for p, t in zip(ps, ts)]
        ts = [pltpu.roll(p, 32, 1) for p in ps]
        ls = []
        for w, (p, t) in enumerate(zip(ps, ts)):
            p = p + t
            if r < DIL * w:
                row = r + jax.lax.broadcasted_iota(jnp.int32, (RA, 128), 0)
                p = jnp.where(row >= DIL * w, p, -1e30)
            ls.append(p)
        m = functools.reduce(jnp.maximum, ls)
        if CH == 4:
            settok(m)
        es = [jnp.exp2(l - m) for l in ls]
        inv = pl.reciprocal(functools.reduce(jnp.add, es), approx=True)
        if CH == 2:
            settok(inv)
        oprev = None
        for a in range(NT):
            o = None
            for w in range(WIN):
                vv = v_s[a, pl.ds(HALO + r - DIL * w, RA), :]
                if w == 0 and LV and oprev is not None:
                    vv = link(vv, oprev)
                t = es[w] * vv
                o = t if o is None else o + t
            oprev = o
            o_s[pl.ds(r // 2, RA // 2), pl.ds(a * 128, 128)] = pltpu.bitcast(
                (o * inv).astype(jnp.bfloat16), jnp.uint32)
        if CH == 1:
            settok(o)

    def wo_mm(s0, n):
        wo = pltpu.bitcast(wo_p[...], jnp.bfloat16)
        lhs = pltpu.bitcast(o_s[pl.ds(s0 // 2, n // 2), :], jnp.bfloat16)
        y = jnp.dot(lhs, wo, preferred_element_type=jnp.float32)
        for a in range(NT):
            h_s[a, pl.ds(s0, n), :] = y[:, a * 128:(a + 1) * 128]

    st = {'best': jnp.full((RA, 1), -jnp.inf, jnp.float32), 'besti': jnp.zeros((RA, 1), jnp.int32)}

    def postc(j):
        r = j * RA
        xs = xtiles(r)
        xs[0] = dep(xs[0])
        hs = [xs[a] + h_s[a, pl.ds(r, RA), :] for a in range(NT)]
        for a in range(NT):
            h_s[a, pl.ds(r, RA), :] = hs[a]
        s3 = lsum([h * w for h, w in zip(hs, wrs)])
        m, rs = stats(hs)
        settok(rs if TP == 0 else m)
        rr = rs * (s3 - m * wsum)
        rowi = r + jax.lax.broadcasted_iota(jnp.int32, (RA, 1), 0)
        upd = rr > st['best']
        st['best'] = jnp.where(upd, rr, st['best'])
        st['besti'] = jnp.where(upd, rowi, st['besti'])
        for a in range(NT):
            out_v[pl.ds(r, RA), pl.ds(a * 128, 128)] = (hs[a] + (hs[a] - m) * rs).astype(jnp.bfloat16)

    def blk(j):
        r = j * RA
        return max(b for b in range(NBK) if STARTS[b] <= r)

    x_cp[0].wait()
    nl = 0
    while nl * RA < BLOCKS[0]:
        ln1c(nl)
        chain['t'] = None
        nl += 1
    for kt in range(NT + 1):
        if kt < NT:
            w_cp[kt].wait()
        if kt == int(2):
            x_cp[2].start()
            wo_cp.start()
            x_cp[3].start()
        if kt == NT:
            for jx in range(4, NX):
                x_cp[jx].start()
        if kt == NT:
            x_cp[1].wait()
        if kt > 0:
            qkv0_part(kt - 1)
        if kt < NT:
            prep_w(kt)
    xw = 2
    npost = 0
    nout = 0
    waited_o = 0
    na = 0
    nbnd = 0
    U = [BLOCKS[0] // 2, BLOCKS[0] // 2] + BLOCKS[1:]
    US = [sum(U[:i]) for i in range(len(U))]
    for u in range(len(U)):
        b = u + 1
        if u in BND:
            while (nout + 1) * XB <= npost * RA:
                o_cp[nout].start()
                nout += 1
            if nbnd == 0:
                wo_cp.wait()
                while xw < 4:
                    x_cp[xw].wait()
                    xw += 1
                prep_wo()
            elif nbnd == 1:
                while xw < NX:
                    x_cp[xw].wait()
                    xw += 1
                wg_cp.start()
                wu_cp.start()
                wd_cp.start()
            else:
                assert waited_o < nout - 1
                o_cp[waited_o].wait()
                waited_o += 1
            nbnd += 1
        if u >= 1:
            assert nbnd >= 1
            wo_mm(US[u - 1], U[u - 1])
        if b < NBK:
            while nl * RA < STARTS[b] + BLOCKS[b]:
                ln1c(nl)
                nl += 1
            qkv(b)
        for c in range(U[u] // RA):
            attc(na)
            na += 1
            lim = max(0, na - U[max(u - 1, 0)] // RA - LP) if u >= 1 else 0
            lim = min(lim, US[u] // RA)
            if nl >= NCK and u >= 2:
                lim = US[u] // RA if c + 1 >= LC else US[u - 1] // RA
            want_ln = min(xw * XB // RA, na + LA)
            k = 0
            if npost < lim:
                postc(npost)
                npost += 1
                k += 1
            if nl < want_ln:
                ln1c(nl)
                nl += 1
                k += 1
            while k < KM and npost < lim:
                postc(npost)
                npost += 1
                k += 1
        assert nl * RA <= xw * XB
    wo_mm(US[-1], U[-1])
    while npost < NCK:
        if DT:
            chain['t'] = None
        postc(npost)
        npost += 1
    while nout < NX:
        o_cp[nout].start()
        nout += 1
    best, besti = st['best'], st['besti']

    rmax = jnp.max(best)
    idx = jnp.min(jnp.where(best == rmax, besti, S))
    idx = jnp.clip(idx, 0, S - 1)
    hrow = [h_s[a, pl.ds(idx, 1), :] for a in range(NT)]
    m, rs = stats(hrow)
    hrow = jnp.concatenate(hrow, axis=1)
    ln2row = (hrow - m) * rs
    xs = jnp.broadcast_to(ln2row, (16, D)).astype(jnp.bfloat16)
    wg_cp.wait()
    wu_cp.wait()
    wd_cp.wait()
    g = jnp.dot(xs, wg_v[...], preferred_element_type=jnp.float32)
    u = jnp.dot(xs, wu_v[...], preferred_element_type=jnp.float32)
    act = (g * jax.nn.sigmoid(g) * u).astype(jnp.bfloat16)
    y = jnp.dot(act, wd_v[...], preferred_element_type=jnp.float32)
    y = y * jax.nn.sigmoid(jnp.full((16, D), rmax, jnp.float32))
    newrow = hrow + ln2row + y[0:1]
    for i in range(waited_o, NX):
        o_cp[i].wait()
    base = pl.multiple_of((idx // 16) * 16, 16)
    tile = out_v[pl.ds(base, 16), :].astype(jnp.float32)
    rr = base + jax.lax.broadcasted_iota(jnp.int32, (16, D), 0)
    tile = jnp.where(rr == idx, jnp.broadcast_to(newrow, (16, D)), tile)
    out_v[pl.ds(base, 16), :] = tile.astype(jnp.bfloat16)
    cp = pltpu.make_async_copy(out_v.at[pl.ds(base, 16), :], out_hbm.at[pl.ds(base, 16), :], osem.at[0])
    cp.start()
    cp.wait()


@jax.jit
def pallas_sequential_preLN__sliding_local_dilated__moe_arch_mod__prompt_kernel(
    A_x, A_wqkv, A_wo, B_x, B_w_r, B_w_gate, B_w_up, B_w_down,
):
    del B_x
    any_spec = pl.BlockSpec(memory_space=pl.ANY)
    out = pl.pallas_call(
        _kernel,
        out_shape=jax.ShapeDtypeStruct((S, D), jnp.bfloat16),
        in_specs=[any_spec, any_spec, any_spec, pl.BlockSpec(memory_space=pltpu.VMEM),
                  any_spec, any_spec, any_spec],
        out_specs=any_spec,
        scratch_shapes=[
            pltpu.VMEM((S, D), jnp.bfloat16),
            pltpu.VMEM((D, 3 * D), jnp.bfloat16),
            pltpu.VMEM((NT, 960, 128), jnp.uint32),
            pltpu.VMEM((960, D), jnp.uint32),
            pltpu.VMEM((D, D), jnp.bfloat16),
            pltpu.VMEM((NT, 320, 128), jnp.uint32),
            pltpu.VMEM((320, D), jnp.uint32),
            pltpu.VMEM((S // 2, D), jnp.uint32),
            pltpu.VMEM((NT, S, 128), jnp.float32),
            pltpu.VMEM((NT, HALO + S, 128), jnp.float32),
            pltpu.VMEM((NT, HALO + S, 128), jnp.float32),
            pltpu.VMEM((S // 2, D), jnp.uint32),
            pltpu.VMEM((NT, S, 128), jnp.float32),
            pltpu.VMEM((S, D), jnp.bfloat16),
            pltpu.VMEM((D, F), jnp.bfloat16),
            pltpu.VMEM((D, F), jnp.bfloat16),
            pltpu.VMEM((F, D), jnp.bfloat16),
            pltpu.SemaphoreType.DMA((NX,)),
            pltpu.SemaphoreType.DMA((NT,)),
            pltpu.SemaphoreType.DMA((4,)),
            pltpu.SemaphoreType.DMA((NX,)),
        ],
        compiler_params=pltpu.CompilerParams(vmem_limit_bytes=100 * 1024 * 1024),
    )(A_x.reshape(S, D), A_wqkv, A_wo, B_w_r, B_w_gate, B_w_up, B_w_down)
    return out.reshape(1, S, D)
```
